```python
import jax
import jax.numpy as jnp

def _softmax(x, axis=-1):
    return jax.nn.softmax(x, axis=axis)
def _gelu(x):
    return jax.nn.gelu(x, approximate=True)
def _silu(x):
    return jax.nn.silu(x)
def _sigmoid(x):
    return jax.nn.sigmoid(x)
def _layernorm(x, axis=-1, eps=1e-5):
    m = jnp.mean(x, axis=axis, keepdims=True)
    v = jnp.var(x, axis=axis, keepdims=True)
    return (x - m) / jnp.sqrt(v + eps)
def _scatter_add(tgt, idx, src, axis=0):
    return tgt.at[idx].add(src)
def _segment_sum(src, seg, n):
    return jax.ops.segment_sum(src, seg, n)
class _Rng:
    def __init__(self, key):
        self._k = key
    def _next(self):
        self._k, sub = jax.random.split(self._k)
        return sub
    def normal(self, shape):
        return jax.random.normal(self._next(), shape, dtype=jnp.bfloat16)
    def randint(self, lo, hi, shape):
        return jax.random.randint(self._next(), shape, lo, hi, dtype=jnp.int32)
    def uniform(self, shape, lo=0.0, hi=1.0):
        return jax.random.uniform(self._next(), shape, jnp.bfloat16, lo, hi)
    def permutation(self, n):
        return jax.random.permutation(self._next(), n)


kernel_name = 'recurrent_scan__linear_kernel_hedgehog__dense_activation_relu__prompt'

def _fwd_setup_inputs():
    _rng = _Rng(jax.random.key(int.from_bytes(__import__("os").urandom(4), "little")))
    _w = (lambda a: (lambda t: t.astype(jnp.bfloat16) if jnp.issubdtype(t.dtype, jnp.floating) else t)(jnp.asarray(a)))
    def _A_setup():
        B, S, D, H = 1, 2048, 1024, 32
        Dh = D // H
        return {
            "x": _w((lambda *s: _rng.normal(s) * 0.05)(B, S, D)),
            "wqkv": _w((lambda *s: _rng.normal(s) * 0.05)(D, 3 * D)),
            "w_phi": _w((lambda *s: _rng.normal(s) * 0.05)(H, Dh, Dh) * (Dh ** -0.5)),
            "wo": _w((lambda *s: _rng.normal(s) * 0.05)(D, D)),
        }
    _A_in = _A_setup()

    def _B_setup():
        B, S, D, Dff = 1, 2048, 1024, 3584
        return {
            "x": _w((lambda *s: _rng.normal(s) * 0.05)(B, S, D)),
            "w1": _w((lambda *s: _rng.normal(s) * 0.05)(D, Dff)),
            "w2": _w((lambda *s: _rng.normal(s) * 0.05)(Dff, D)),
        }
    _B_in = _B_setup()

    return {
        "A_x": _A_in["x"],
        "A_wqkv": _A_in["wqkv"],
        "A_w_phi": _A_in["w_phi"],
        "A_wo": _A_in["wo"],
        "B_x": _B_in["x"],
        "B_w1": _B_in["w1"],
        "B_w2": _B_in["w2"],
    }

def _fwd_reference(A_x, A_wqkv, A_w_phi, A_wo, B_x, B_w1, B_w2):
    def _A_ref(x, wqkv, w_phi, wo):
        B, S, D = x.shape
        H = 32; Dh = D // H
        qkv = (lambda x, *d: x.transpose(*d))((x @ wqkv).reshape(B, S, 3, H, Dh), 2, 0, 3, 1, 4)
        q, k, v = qkv[0], qkv[1], qkv[2]
        pq = jnp.einsum("bhsd,hdf->bhsf", q, w_phi)
        pk = jnp.einsum("bhsd,hdf->bhsf", k, w_phi)
        phi_q = jnp.concatenate([_softmax(pq, axis=-1), _softmax(-pq, axis=-1)], axis=-1)
        phi_k = jnp.concatenate([_softmax(pk, axis=-1), _softmax(-pk, axis=-1)], axis=-1)
        kv = jnp.einsum("bhsf,bhsd->bhfd", phi_k, v)
        z  = jnp.einsum("bhsf->bhf", phi_k)
        num = jnp.einsum("bhqf,bhfd->bhqd", phi_q, kv)
        den = jnp.einsum("bhqf,bhf->bhq", phi_q, z)[..., None] + 1e-6
        o = num / den
        return (lambda x, *d: x.transpose(*d))(o, 0, 2, 1, 3).reshape(B, S, D) @ wo

    def _B_ref(x, w1, w2):
        h = jnp.einsum("bsd,df->bsf", x, w1)
        zero = jnp.zeros_like(h)
        h = jnp.maximum(h, zero)
        return jnp.einsum("bsf,fd->bsd", h, w2)

    x = A_x
    xn = _layernorm(x, axis=-1)
    s = _A_ref(xn, A_wqkv, A_w_phi, A_wo)
    g = _silu(_B_ref(xn, B_w1, B_w2))
    return x + s * g


def setup_inputs():
    _inp = _fwd_setup_inputs()
    _gk = jax.random.fold_in(jax.random.key(int.from_bytes(__import__("os").urandom(4), "little")), 2**31 - 1)
    _shapes = [[1, 2048, 1024]]
    _dtypes = ['bfloat16']
    _gks = jax.random.split(_gk, len(_shapes))
    _gs = [jax.random.normal(k, s, dtype=jnp.dtype(d)) * 0.05 for k, s, d in zip(_gks, _shapes, _dtypes)]
    _inp["grad_out"] = _gs[0]
    return _inp

def reference(A_x, A_wqkv, A_w_phi, A_wo, B_w1, B_w2, B_x, grad_out):
    _const = dict(B_x=B_x)
    def _f(*_d):
        return _fwd_reference(**{'A_x': _d[0], 'A_wqkv': _d[1], 'A_w_phi': _d[2], 'A_wo': _d[3], 'B_w1': _d[4], 'B_w2': _d[5], **_const})
    _out, _vjp = jax.vjp(_f, A_x, A_wqkv, A_w_phi, A_wo, B_w1, B_w2)
    _grads = _vjp(grad_out)
    _out0 = jnp.asarray(_out)
    return (_out0, *[jnp.asarray(_g) for _g in _grads])
```

```python
import jax
import jax.numpy as jnp
from jax import lax
import jax.experimental.pallas as pl
import jax.experimental.pallas.tpu as pltpu

BF, F32 = jnp.bfloat16, jnp.float32
V = pltpu.VMEM
S, D, H, DH, DFF = 2048, 1024, 32, 32, 3584
T = 512
NT = S // T
U = 256
NU = S // U
C = 512
NC = DFF // C
G = 128
NG = D // G
HG = G // DH
W2_EARLY = 608
P = G // 2


def _nn(a, b):
    return lax.dot_general(a, b, (((1,), (0,)), ((), ())), preferred_element_type=F32)


def _nt(a, b):
    return lax.dot_general(a, b, (((1,), (1,)), ((), ())), preferred_element_type=F32)


def _tn(a, b):
    return lax.dot_general(a, b, (((0,), (0,)), ((), ())), preferred_element_type=F32)


def _quarters(x):
    r, c = x.shape[0] // 2, x.shape[1] // 2
    return x[:r, :c], x[:r, c:], x[r:, :c], x[r:, c:]


def _join(q):
    return jnp.concatenate([jnp.concatenate(q[:2], axis=1), jnp.concatenate(q[2:], axis=1)], axis=0)


def _forms(q, transposed=False):
    a, b, c, d = q
    if transposed:
        b, c = c, b
    fa, fb, fc, fd = (v.astype(F32) for v in (a, b, c, d))
    return [v.astype(BF) for v in (fa + fd, fc + fd, a, d, fa + fb, fc - fa, fb - fd)]


_RHS = (0, 2, 6, 5, 3, 4, 1)
_USE = ("+..+", "..+-", ".+.+", "+.+.", "-+..", "...+", "+...")
PLAIN_RHS, PLAIN_LHS = (1, 4, 3, 2, 0, 6, 5), (3, 2, 4, 1, 0, 6, 5)


def _strassen(dot, lhs, rhs, order=PLAIN_RHS):
    acc = [None] * 4
    for k in order:
        m = dot(lhs[k], rhs[_RHS[k]])
        for q, sign in enumerate(_USE[k]):
            if sign == ".":
                continue
            if acc[q] is None:
                acc[q] = (sign, m)
            elif acc[q][0] == "-":
                acc[q] = (sign, m - acc[q][1])
            else:
                acc[q] = ("+", acc[q][1] + m if sign == "+" else acc[q][1] - m)
    return [v for _, v in acc]


def _slab(ref, e, g):
    half = ref.shape[1] // 2
    if e in (2, 3):
        return (e - 2) * NG // 2 + g, (e - 2) * half
    return NG + 2 * (e if e < 2 else e - 2) + g // 2, g % 2 * half


def _slab_form(ref, e):
    return jnp.concatenate([ref[n, pl.ds(r, ref.shape[1] // 2), :]
                            for n, r in (_slab(ref, e, g) for g in range(NG // 2))], axis=1)


def _build_slab_forms(ref, start, rows):
    half = ref.shape[1] // 2
    for t in range(0, rows, 16):
        r0 = pl.multiple_of(start + t, 16)
        for g in range(NG // 2):
            v = _forms([ref[g + c, pl.ds(r0 + r, 16), :] for r in (0, half) for c in (0, NG // 2)])
            for e in (0, 1, 4, 5, 6):
                n, r = _slab(ref, e, g)
                ref[n, pl.ds(r0 + r, 16), :] = v[e]


def _head_mask(rows, cols):
    r = lax.broadcasted_iota(jnp.int32, (rows, cols), 0)
    c = lax.broadcasted_iota(jnp.int32, (rows, cols), 1)
    return (r // DH) == (c % rows // DH)


def _seg(a):
    return a.reshape(a.shape[0] // DH, DH, a.shape[1])


def _unseg(a):
    return a.reshape(a.shape[0] * DH, a.shape[2])


def _fold_lanes(a):
    out = a[:, :128]
    for c in range(1, a.shape[1] // 128):
        out = out + a[:, c * 128:(c + 1) * 128]
    return out


def _tile_lanes(a, n):
    return jnp.concatenate([a] * (n // a.shape[1]), axis=1)


def _zip(a, b):
    return jnp.concatenate([a[:2], b[:2], a[2:], b[2:]], axis=0)


def _unzip(r):
    return jnp.concatenate([r[0:2], r[4:6]], axis=0), jnp.concatenate([r[2:4], r[6:8]], axis=0)


def _pairs(f):
    return jnp.concatenate([f(0), f(1)], axis=0)


def _dual_softmax(p):
    p3 = _seg(p)
    ep = jnp.exp(p3 - jnp.max(p3, axis=1, keepdims=True))
    em = jnp.exp(jnp.min(p3, axis=1, keepdims=True) - p3)
    return _zip(ep * (1.0 / jnp.sum(ep, axis=1, keepdims=True)), em * (1.0 / jnp.sum(em, axis=1, keepdims=True)))


def _dual_softmax_bwd(phi, dphi):
    p3, d3 = _seg(phi), _seg(dphi)
    rp, rm = _unzip(p3 * (d3 - jnp.sum(p3 * d3, axis=1, keepdims=True)))
    return _unseg(rp - rm)


def _ln(x):
    xc = x - jnp.mean(x, axis=-1, keepdims=True)
    rstd = lax.rsqrt(jnp.mean(xc * xc, axis=-1, keepdims=True) + 1e-5)
    return xc * rstd, rstd


def _kernel(x_hbm, wqkv_hbm, wphi_hbm, wo_hbm, w1_hbm, w2_hbm, dy_hbm,
            out_hbm, dx_hbm, dwqkv_hbm, dwphi_hbm, dwo_hbm, dw1_hbm, dw2_hbm,
            dy_v, rstd_v, w1_v, wo_v, wq_v, wk_v, wv_v, wts_v, bd_v, bdt_v, h_v, pk_v, dq_v, vt_v,
            kv_a, z_a, kv_v, kvt_v, z_v, st1_v, st2_v, wphi_v, dwphi_a, xs_v,
            sem_x, sem_dy, sem_w1, sem_w2, sem_wo, sem_w, sem_o, sem_g, sem_p):
    w_v = (wq_v, wk_v, wv_v)

    def cp_w1(j):
        return pltpu.make_async_copy(w1_hbm.at[:, pl.ds(j * C, C)], w1_v.at[j], sem_w1.at[j])

    def cp_w(j):
        return pltpu.make_async_copy(wqkv_hbm.at[:, pl.ds(j * D, D)], w_v[j], sem_w.at[0])

    def cp_dw(j):
        return pltpu.make_async_copy(w_v[j], dwqkv_hbm.at[:, pl.ds(j * D, D)], sem_g.at[0])

    cp_wphi = pltpu.make_async_copy(wphi_hbm, wphi_v, sem_p.at[0])
    cp_dwphi = pltpu.make_async_copy(wphi_v, dwphi_hbm, sem_p.at[0])
    cp_wo = [pltpu.make_async_copy(wo_hbm.at[:, pl.ds(g * G, G)], wo_v.at[g], sem_wo.at[0]) for g in range(NG)]
    cp_dwo = [pltpu.make_async_copy(wo_v.at[g], dwo_hbm.at[:, pl.ds(g * G, G)], sem_wo.at[0]) for g in range(NG)]

    cp_dy = pltpu.make_async_copy(dy_hbm, dy_v, sem_dy.at[0])

    def cp_out(i, dst):
        return pltpu.make_async_copy(st2_v.at[i % 2], dst.at[pl.ds(i * U, U)], sem_o.at[i % 2])

    def cp_dw2(c):
        return pltpu.make_async_copy(st2_v.at[2 + c % 2], dw2_hbm.at[pl.ds(c * U, U)], sem_o.at[4 + c % 2])

    def cp_dw1(j):
        return pltpu.make_async_copy(st1_v.at[j % 2], dw1_hbm.at[:, pl.ds(j * U, U)], sem_o.at[2 + j % 2])

    def finalize(g):
        kvt = [jnp.where(_head_mask(P, G), kv_a[g, pl.ds(e * P, P)], 0.0) for e in range(2)]
        zero = jnp.zeros((P, G), F32)
        kvt_v[g] = jnp.concatenate(kvt, axis=0).astype(BF)
        kv_v[g] = jnp.concatenate([jnp.concatenate([kvt[0], zero], axis=0).T,
                                   jnp.concatenate([zero, kvt[1]], axis=0).T], axis=0).astype(BF)
        z_v[g] = jnp.broadcast_to(jnp.sum(z_a[g], axis=1, keepdims=True), (2 * G, G))

    def mlp_phases(w2_v, dms_v, dwo_a):
        cp_w2_early, cp_w2 = (
            [pltpu.make_async_copy(w2_hbm.at[pl.ds(r + r0, n), pl.ds(g * G, G)], w2_v.at[g, pl.ds(r + r0, n)],
                                   sem_w2.at[0]) for r in (0, DFF // 2) for g in range(NG)]
            for r0, n in ((0, W2_EARLY), (W2_EARLY, DFF // 2 - W2_EARLY)))

        def forward(x_v, pq_v, ot_v, rden_v):
            def cp_x(u):
                return pltpu.make_async_copy(x_hbm.at[pl.ds(u * U, U)], x_v.at[pl.ds(u * U, U)], sem_x.at[u])

            def cp_x0(q):
                return pltpu.make_async_copy(x_hbm.at[pl.ds(q * G, G)], x_v.at[pl.ds(q * G, G)], sem_dy.at[q])

            def h_tile(xn, i, j):
                h = _nn(xn, w1_v[j])
                h_v[j, pl.ds(pl.multiple_of(i * T, T), T), :] = jnp.where(h < 0, -0.0, jnp.abs(h)).astype(BF)

            def xn_tile(i):
                return jnp.concatenate([dms_v[i, pl.ds(k * T, T), :] for k in range(2)], axis=1)

            def ln_rows(r0, n):
                rows = pl.ds(r0, n)
                xn, rstd = _ln(x_v[rows, :].astype(F32))
                for k in range(2):
                    dms_v[r0 // T, pl.ds(pl.multiple_of(k * T + r0 % T, n), n), :] = (
                        xn[:, k * D // 2:(k + 1) * D // 2].astype(BF))
                xs_v[7 + r0 // T, pl.ds(pl.multiple_of(r0 % T, n), n), :] = xn.astype(BF)
                rstd_v[rows, :] = jnp.broadcast_to(rstd, (n, G))

            for q in range(T // G):
                cp_x0(q).start()
            cp_w1(0).start()

            def first_rows(q, _):
                cp_x0(q).wait()
                ln_rows(pl.multiple_of(q * G, G), G)

            def block_diag(g):
                w4 = _unseg(wphi_v[pl.ds(g * HG, HG)].astype(F32))
                bd = jnp.where(_head_mask(G, G), _tile_lanes(w4, G), 0.0)
                bd_v[g] = bd.astype(BF)
                bdt_v[g] = bd.T.astype(BF)

            def clear(g, _):
                kv_a[g] = jnp.zeros((G, G), F32)
                z_a[g] = jnp.zeros((2 * G, G), F32)

            lax.fori_loop(0, NG, clear, None)
            lax.fori_loop(0, T // G, first_rows, None)

            def up_first(j, _):
                cp_w1(j).wait()

                @pl.when(j + 1 < NC)
                def _():
                    cp_x(j + 2).start()
                    cp_w1(j + 1).start()

                @pl.when(j + 1 == NC)
                def _():
                    for cp in [cp_wphi] + cp_w2_early[5:]:
                        cp.start()

                @pl.when(j + 2 == NC)
                def _():
                    for cp in cp_w2_early[:5]:
                        cp.start()

                @pl.when(j >= 1)
                def _():
                    cp_x(j + 1).wait()

                xn = xn_tile(0)
                ln_rows(pl.multiple_of((j + 1) * U, U), U)
                h_tile(xn, 0, j)

            lax.fori_loop(0, NC, up_first, None)
            for cp in [cp_wphi] + cp_w2_early:
                cp.wait()
            for cp in cp_w2 + cp_wo:
                cp.start()

            def up_rest(i, _):
                @pl.when(i == 2)
                def _():
                    for cp in cp_w2 + cp_wo:
                        cp.wait()
                    for j in range(3):
                        cp_w(j).start()
                    cp_dy.start()

                _build_slab_forms(w2_v, (i - 1) * (W2_EARLY - 16), W2_EARLY)
                for k in range(3):
                    u = jnp.minimum(3 * (i - 1) + k, NU - 1)
                    block_diag(u)
                    for c in range(0, D // 2, G):
                        for e in range(7):
                            q = [xs_v[7 + u // 2, pl.ds(pl.multiple_of(u % 2 * U + r, G), G), pl.ds(c + c0, G)]
                                 for r in (0, G) for c0 in (0, D // 2)]
                            xs_v[e, pl.ds(c, G), pl.ds(pl.multiple_of(u * G, G), G)] = _forms(q, True)[e].T
                for j in range(NC):
                    h_tile(xn_tile(i), i, j)

            lax.fori_loop(1, NT, up_rest, None)

            for j in range(3):
                cp_w(j).wait()

            def fold(k, g):
                w = [w_v[k][:, pl.ds(gg * G, G)] for gg in (g, g + NG // 2)]
                if k == 2:
                    forms = [v.T for v in _forms(_quarters(jnp.concatenate(w, axis=1)), True)]
                else:
                    forms = _forms(_quarters(jnp.concatenate(
                        [_nt(bdt_v[g], w[0]), _nt(bdt_v[g + NG // 2], w[1])], axis=0)))
                for e, v in enumerate(forms):
                    wts_v[e, pl.ds(k * D // 2 + g * G, G), :] = v

            def project(k, xs):
                return _join(_strassen(lambda e, b: _nn(wts_v[e, pl.ds(k * D // 2, D // 2), :], b), range(7), xs))

            for g in range(NG // 2):
                fold(1, g)
                fold(2, g)

            def kv_tile(i, _):
                xs = [xs_v[e, :, pl.ds(pl.multiple_of(i * U, U), U)] for e in range(7)]
                dwo_a[pl.ds(pl.multiple_of(i * U, U), U), :] = jnp.zeros((U, D), F32)
                _build_slab_forms(wo_v, i * G, G)
                pk, vt = (jnp.concatenate([p[:, r:r + G] for r in (0, 2 * G, G, 3 * G)], axis=1)
                          for p in (project(1, xs), project(2, xs).astype(BF)))
                for k in range(T // U):
                    vt_v[i * (T // U) + k] = vt[:, k * U:(k + 1) * U]
                for g in range(NG):
                    phi = _unseg(_dual_softmax(pk[g * G:(g + 1) * G]))
                    z_a[g] += _fold_lanes(phi)
                    phi = phi.astype(BF)
                    pk_v[i, g] = phi
                    kv_a[g] += _pairs(lambda e: _nt(vt[g * G + e * P:g * G + (e + 1) * P], phi[e * G:(e + 1) * G]))

            lax.fori_loop(0, NT, kv_tile, None)

            for g in range(NG):
                if g % 2 == 0:
                    fold(0, g // 2)
                finalize(g)
            kv_a[...] = jnp.zeros_like(kv_a)
            z_a[...] = jnp.zeros_like(z_a)
            cp_dy.wait()

            def query_tile(u, _):
                @pl.when(u >= 2)
                def _():
                    cp_out(u - 2, out_hbm).wait()

                rows = pl.ds(pl.multiple_of(u * U, U), U)
                pq = project(0, [xs_v[e, :, pl.ds(pl.multiple_of(u * G, G), G)] for e in range(7)])
                h = jnp.concatenate([h_v[j, rows, :] for j in range(NC)], axis=1)

                def group(g):
                    phi3 = _dual_softmax(pq[g * G:(g + 1) * G])
                    phi = _unseg(phi3)
                    pq_v[g] = phi
                    tp, tm = _unzip(phi3 * _seg(_tile_lanes(z_v[g], U)))
                    rden = 1.0 / (jnp.sum(tp + tm, axis=1, keepdims=True) + 1e-6)
                    rden = _unseg(jnp.broadcast_to(rden, (HG, DH, U)))
                    rden_v[g] = rden
                    ot_v[g] = _pairs(lambda e: _nn(kvt_v[g, pl.ds(e * P, P)], phi[e * G:(e + 1) * G].astype(BF))) * rden

                steps = iter(((0,), (1,), (), (2,), (3,), (4,), (), (), (5,), (6,), (7,), (), (), ()))
                hs = _forms(_quarters(h))

                def down(c):
                    def dot(a, e):
                        m = _nn(a, _slab_form(w2_v, e)[:, c * U:(c + 1) * U])
                        for g in next(steps):
                            group(g)
                        return m
                    return _strassen(dot, hs, range(7), PLAIN_LHS)

                m = _join([jnp.concatenate(q, axis=1) for q in zip(down(0), down(1))])
                ot = ot_v[...].reshape(D, U)
                s = _join(_strassen(lambda o, e: _tn(o, _slab_form(wo_v, e)),
                                    _forms(_quarters(ot), True), range(7), PLAIN_LHS))
                ot = ot.astype(BF)
                sig = 1.0 / (1.0 + jnp.exp(-m))
                gate = m * sig
                dy = dy_v[rows, :].astype(F32)
                ds = dy * gate
                st2_v[u % 2] = (x_v[rows, :].astype(F32) + s * gate).astype(BF)
                cp_out(u, out_hbm).start()
                for e, v in enumerate(_forms(_quarters(dy * s * (sig + gate * (1.0 - sig))))):
                    dms_v[e, pl.ds(pl.multiple_of(u * G, G), G), :] = v
                dot = _join(_strassen(lambda e, b: _nt(_slab_form(wo_v, e), b), range(7), _forms(_quarters(ds), True),
                                      (1, 3, 5, 4, 2, 0, 6)))
                ds = ds.astype(BF)
                for g in range(NG):
                    dnum = dot[g * G:(g + 1) * G] * rden_v[g]
                    dden = -jnp.sum(_seg(dnum * ot_v[g]), axis=1, keepdims=True)
                    dden = jnp.broadcast_to(dden, (HG, DH, U))
                    dden = _unseg(_zip(dden, dden))
                    phi = pq_v[g]
                    dnum = dnum.astype(BF)
                    dphi = _nn(kv_v[g], dnum) + _tile_lanes(z_v[g], U) * dden
                    z_a[g] += _fold_lanes(phi * dden)
                    dq_v[u, pl.ds(g * G, G), :] = _dual_softmax_bwd(phi, dphi).astype(BF)
                    kv_a[g] += _pairs(lambda e: _nt(dnum[e * P:(e + 1) * P], phi[e * G:(e + 1) * G].astype(BF)))
                    dwo_a[pl.ds(g * G, G), :] += _nn(ot[g * G:(g + 1) * G], ds)

            lax.fori_loop(0, NU, query_tile, None)

        pl.run_scoped(forward, V((S, D), BF), V((NG, 2 * G, U), F32), V((NG, G, U), F32), V((NG, G, U), F32))

        def mlp_bwd(c, _):
            @pl.when(c >= 2)
            def _():
                cp_dw2(c - 2).wait()
                cp_dw1(c - 2).wait()

            j, cols = c // (C // U), pl.ds(pl.multiple_of(c % (C // U) * U, U), U)
            h = _quarters(jnp.concatenate([h_v[j, pl.ds(u * U + r, G), cols] for r in (0, G) for u in range(NU)],
                                          axis=0).astype(F32))
            w2 = jnp.concatenate([w2_v[g, pl.ds(pl.multiple_of(c * U, U), U), :] for g in range(NG)], axis=1)
            dh = []
            for hq, dq in zip(h, _strassen(_nt, dms_v, _forms(_quarters(w2), True))):
                bits = pltpu.bitcast(hq, jnp.int32)
                dh.append(jnp.where(bits > 0, dq, jnp.where(bits == 0, 0.5 * dq, 0.0)))
            st2_v[2 + c % 2] = _join(_strassen(_tn, _forms(h, True), dms_v, PLAIN_LHS)).astype(BF)
            st1_v[c % 2] = _join(_strassen(_nn, xs_v, _forms(dh))).astype(BF)
            dh = _join(dh).astype(BF)
            for k, r0 in enumerate(u * U + r for r in (0, G) for u in range(NU)):
                h_v[j, pl.ds(r0, G), cols] = dh[k * G:(k + 1) * G]
            g = jnp.minimum(c, NG - 1)
            finalize(g)
            wo_v[g] = dwo_a[:, pl.ds(pl.multiple_of(g * G, G), G)].astype(BF)

            cp_dw2(c).start()
            cp_dw1(c).start()

        lax.fori_loop(0, DFF // U, mlp_bwd, None)

    pl.run_scoped(mlp_phases, V((NG + 10, DFF, G), BF), V((7, S // 2, D // 2), BF), V((D, D), F32))
    for cp in cp_dwo:
        cp.start()

    def backward(dk_v, dv_v, dxn_v, w1s_v):
        def proj_grad(dp_v, r0, n, lhs=lambda e: xs_v[e]):
            rows = pl.ds(pl.multiple_of(r0, n), n)
            dp = jnp.concatenate([dp_v[u, rows, pl.ds(r, G)] for r in (0, G) for u in range(NU)], axis=1)
            return _join(_strassen(lambda e, b: _nt(lhs(e), b), range(7), _forms(_quarters(dp), True))).astype(BF)

        def unfold(wp_v, g, dw):
            grp = pl.ds(pl.multiple_of(g * G, G), G)
            dphi_w = _tn(wp_v[:, grp], dw)
            for r in range(4):
                wp_v[pl.ds(r * U, U), grp] = _nt(dw[r * U:(r + 1) * U], bd_v[g]).astype(BF)
            return dphi_w

        def kv_bwd(a, _):
            def per_tile(b, f):
                for g in (4 * a + 2 * b, 4 * a + 2 * b + 1):
                    for u in range(NU):
                        f(g, u, pl.ds(pl.multiple_of(g * G, G), G), pk_v[u // (T // U), g, :, pl.ds(u % (T // U) * U, U)])

            def dk(g, u, grp, phi):
                dphi = _nn(kv_v[g], vt_v[u, grp, :]) + _tile_lanes(z_v[g], U)
                dk_v[u, grp, :] = _dual_softmax_bwd(phi.astype(F32), dphi).astype(BF)

            def dv(g, u, grp, phi):
                dv_v[u, grp, :] = _pairs(lambda e: _nn(kvt_v[g, pl.ds(e * P, P)], phi[e * G:(e + 1) * G])).astype(BF)

            for e in range(7):
                half = pl.ds(pl.multiple_of(a * U, U), U)
                w1s_v[e, half, pl.ds(DFF // 2, G)] = xs_v[e, half, pl.ds(0, G)]
            for b in range(2):
                per_tile(b, dk)
                dw = proj_grad(dq_v, (4 * a + 2 * b) * G, 2 * G)
                per_tile(b, dv)
                for e in range(2):
                    g = 4 * a + 2 * b + e
                    dwphi_a[g] = unfold(wq_v, g, dw[:, e * G:(e + 1) * G])

        def kv_wgrad(a, _):
            def after(pieces):
                def lhs(e):
                    col = []
                    for r in range(0, D // 2, P):
                        next(pieces, None)
                        col.append(w1s_v[e, pl.ds(r, P), pl.ds(DFF // 2, G)])
                    return jnp.concatenate([jnp.concatenate(col, axis=0), xs_v[e, :, pl.ds(G, S // 2 - G)]], axis=1)
                return lhs

            dw = proj_grad(dk_v, 2 * a * G, 2 * G, after(w1_forms(a)))
            wv_v[:, pl.ds(pl.multiple_of(2 * a * G, 2 * G), 2 * G)] = proj_grad(dv_v, 2 * a * G, 2 * G)
            for e in range(2):
                g = 2 * a + e
                dphi_w = dwphi_a[g] + unfold(wk_v, g, dw[:, e * G:(e + 1) * G])
                for b in range(HG):
                    wphi_v[g * HG + b] = dphi_w[b * DH:(b + 1) * DH, b * DH:(b + 1) * DH].astype(BF)

        def w1_forms(a):
            for k in range(DFF // 2 // U):
                for t in range(0, G, 16):
                    r0 = pl.multiple_of(a * G + t, 16)
                    q = [w1_v[c // C, pl.ds(r0 + r, 16), pl.ds(c % C, U)]
                         for r in (0, D // 2) for c in (k * U, DFF // 2 + k * U)]
                    for e, v in enumerate(_forms(q, True)):
                        w1s_v[e, pl.ds(r0, 16), pl.ds(k * U, U)] = v
                    yield

        def tag(e):
            return 2 + e // 4, pl.ds(e % 4 // 2 * G, G), pl.ds(e % 2 * (D // 2), D // 2)

        lax.fori_loop(0, NG // 4, kv_bwd, None)
        lax.fori_loop(0, NG // 2, kv_wgrad, None)
        cp_dwphi.start()
        for u in range(NU - 2, NU):
            cp_out(u, out_hbm).wait()
        for j in range(3):
            cp_dw(j).start()
        for c in range(DFF // U - 2, DFF // U):
            cp_dw2(c).wait()
            cp_dw1(c).wait()

        def dx_rows(u, r0, n):
            rows = pl.ds(pl.multiple_of(u * U + r0, 16), n)
            dxn = dxn_v[pl.ds(r0, n), :]
            xn = xs_v[7 + u // 2, pl.ds(pl.multiple_of(u % 2 * U + r0, 16), n), :].astype(F32)
            rstd = _tile_lanes(rstd_v[rows, :], D)
            dx = rstd * (dxn - jnp.mean(dxn, axis=-1, keepdims=True)
                         - xn * jnp.mean(dxn * xn, axis=-1, keepdims=True))
            st2_v[u % 2, pl.ds(r0, n), :] = (dy_v[rows, :].astype(F32) + dx).astype(BF)

        def dx_tile(u, _):
            @pl.when(u >= 3)
            def _():
                cp_out(u - 3, dx_hbm).wait()

            pieces = iter(range(0, U, 32))

            def dot(lhs, e):
                dx_rows(jnp.maximum(u - 1, 0), next(pieces), 32)
                wt = jnp.concatenate([wts_v[e, pl.ds(0, 3 * D // 2 - G), :], st2_v[tag(e)]], axis=0)
                return _nt(lhs[0], w1s_v[e, :, pl.ds(0, DFF // 2)]) + _tn(lhs[1], wt)

            rows = pl.ds(pl.multiple_of(u * U, U), U)
            dh = _forms(_quarters(jnp.concatenate([h_v[j, rows, :] for j in range(NC)], axis=1)))
            dp = _forms(_quarters(jnp.concatenate(
                [ref[u, pl.ds(r, D // 2), :] for r in (0, D // 2) for ref in (dq_v, dk_v, dv_v)], axis=0)), True)
            dxn = _join(_strassen(dot, list(zip(dh, dp)), range(7), PLAIN_LHS))
            dx_rows(jnp.maximum(u - 1, 0), next(pieces), 32)
            dxn_v[...] = dxn

            @pl.when(u >= 1)
            def _():
                cp_out(u - 1, dx_hbm).start()

        dxn_v[...] = jnp.zeros_like(dxn_v)
        for e in range(7):
            st2_v[tag(e)] = wts_v[e, pl.ds(3 * D // 2 - G, G), :]
        lax.fori_loop(0, NU, dx_tile, None)
        cp_out(NU - 3, dx_hbm).wait()
        last = [pltpu.make_async_copy(st2_v.at[1, pl.ds(r, G)], dx_hbm.at[pl.ds(S - U + r, G)], sem_o.at[1])
                for r in (0, G)]
        for k, cp in enumerate(last):
            dx_rows(NU - 1, k * G, G)
            cp.start()
        for cp in cp_dwo:
            cp.wait()
        cp_dwphi.wait()
        for j in range(3):
            cp_dw(j).wait()
        for cp in [cp_out(NU - 2, dx_hbm)] + last:
            cp.wait()

    pl.run_scoped(backward, V((NU, D, U), BF), V((NU, D, U), BF), V((U, D), F32),
                  V((7, D // 2, DFF // 2 + G), BF))


@jax.jit
def pallas_recurrent_scan__linear_kernel_hedgehog__dense_activation_relu__prompt_kernel(
    A_x: jax.Array,
    A_wqkv: jax.Array,
    A_w_phi: jax.Array,
    A_wo: jax.Array,
    B_x: jax.Array,
    B_w1: jax.Array,
    B_w2: jax.Array,
    grad_out: jax.Array,
):
    del B_x
    hbm = pl.BlockSpec(memory_space=pl.ANY)
    sds = jax.ShapeDtypeStruct
    dma = pltpu.SemaphoreType.DMA
    out, dx, dwqkv, dwphi, dwo, dw1, dw2 = pl.pallas_call(
        _kernel,
        out_shape=(sds((S, D), BF), sds((S, D), BF), sds((D, 3 * D), BF), sds((H, DH, DH), BF),
                   sds((D, D), BF), sds((D, DFF), BF), sds((DFF, D), BF)),
        in_specs=[hbm] * 7,
        out_specs=(hbm,) * 7,
        scratch_shapes=[
            V((S, D), BF), V((S, G), F32),
            V((NC, D, C), BF), V((NG + 10, D, G), BF), *[V((D, D), BF)] * 3,
            V((7, 3 * D // 2, D // 2), BF),
            V((NG, G, G), BF), V((NG, G, G), BF),
            V((NC, S, C), BF), V((NT, NG, 2 * G, T), BF),
            V((NU, D, U), BF), V((NU, D, U), BF),
            V((NG, G, G), F32), V((NG, 2 * G, G), F32),
            V((NG, 2 * G, G), BF), V((NG, G, G), BF), V((NG, 2 * G, G), F32),
            V((2, D, U), BF), V((4, U, D), BF),
            V((H, DH, DH), BF), V((NG, G, G), F32),
            V((7 + NT, D // 2, S // 2), BF),
            dma((NU,)), dma((NT,)), dma((NC,)), dma((1,)), dma((1,)), dma((1,)), dma((6,)), dma((1,)), dma((1,)),
        ],
        compiler_params=pltpu.CompilerParams(vmem_limit_bytes=127 * 2**20),
    )(A_x.reshape(S, D), A_wqkv, A_w_phi, A_wo, B_w1, B_w2, grad_out.reshape(S, D))
    return out.reshape(1, S, D), dx.reshape(1, S, D), dwqkv, dwphi, dwo, dw1, dw2
```
